```python
import jax
import jax.numpy as jnp

def _softmax(x, axis=-1):
    return jax.nn.softmax(x, axis=axis)
def _gelu(x):
    return jax.nn.gelu(x, approximate=True)
def _silu(x):
    return jax.nn.silu(x)
def _sigmoid(x):
    return jax.nn.sigmoid(x)
def _layernorm(x, axis=-1, eps=1e-5):
    m = jnp.mean(x, axis=axis, keepdims=True)
    v = jnp.var(x, axis=axis, keepdims=True)
    return (x - m) / jnp.sqrt(v + eps)
def _scatter_add(tgt, idx, src, axis=0):
    return tgt.at[idx].add(src)
def _segment_sum(src, seg, n):
    return jax.ops.segment_sum(src, seg, n)
class _Rng:
    def __init__(self, key):
        self._k = key
    def _next(self):
        self._k, sub = jax.random.split(self._k)
        return sub
    def normal(self, shape):
        return jax.random.normal(self._next(), shape, dtype=jnp.bfloat16)
    def randint(self, lo, hi, shape):
        return jax.random.randint(self._next(), shape, lo, hi, dtype=jnp.int32)
    def uniform(self, shape, lo=0.0, hi=1.0):
        return jax.random.uniform(self._next(), shape, jnp.bfloat16, lo, hi)
    def permutation(self, n):
        return jax.random.permutation(self._next(), n)


kernel_name = 'gated_mix__compressed_kv_cla__ssm_conv_s5__prompt'

def setup_inputs():
    _rng = _Rng(jax.random.key(int.from_bytes(__import__("os").urandom(4), "little")))
    _w = (lambda a: (lambda t: t.astype(jnp.bfloat16) if jnp.issubdtype(t.dtype, jnp.floating) else t)(jnp.asarray(a)))
    def _A_setup():
        B, H, Sq, Sk, D, M = 1, 16, 2048, 2048, 256, 448
        Dc = 4 * D
        return {
            "x": _w((lambda *s: _rng.normal(s) * 0.05)(B, Sq, M)),
            "c_kv": _w((lambda *s: _rng.normal(s) * 0.05)(B, Sk, Dc)),
            "w_q": _w((lambda *s: _rng.normal(s) * 0.05)(M, H, D) * (M ** -0.5)),
            "w_uk": _w((lambda *s: _rng.normal(s) * 0.05)(Dc, H, D) * (Dc ** -0.5)),
            "w_uv": _w((lambda *s: _rng.normal(s) * 0.05)(Dc, H, D) * (Dc ** -0.5)),
            "w_o": _w((lambda *s: _rng.normal(s) * 0.05)(H, D, M) * ((H * D) ** -0.5)),
        }
    _A_in = _A_setup()

    def _B_setup():
        B, S, D = 1, 2048, 448
        P = D
        Lambda_re = -0.5 * jnp.exp((lambda *s: _rng.normal(s) * 0.05)(P))
        Lambda_im = (lambda *s: _rng.normal(s) * 0.05)(P) * 1.0
        B_re = (lambda *s: _rng.normal(s) * 0.05)(P, D) * (D ** -0.5)
        B_im = (lambda *s: _rng.normal(s) * 0.05)(P, D) * (D ** -0.5)
        C_re = (lambda *s: _rng.normal(s) * 0.05)(D, P) * (P ** -0.5)
        C_im = (lambda *s: _rng.normal(s) * 0.05)(D, P) * (P ** -0.5)
        log_dt = (lambda *s: _rng.normal(s) * 0.05)(P) * 0.3 - 2.0
        Dskip = (lambda *s: _rng.normal(s) * 0.05)(D)
        return {
            "x": _w((lambda *s: _rng.normal(s) * 0.05)(B, S, D)),
            "Lambda_re": _w(Lambda_re),
            "Lambda_im": _w(Lambda_im),
            "B_re": _w(B_re),
            "B_im": _w(B_im),
            "C_re": _w(C_re),
            "C_im": _w(C_im),
            "log_dt": _w(log_dt),
            "Dskip": _w(Dskip),
        }
    _B_in = _B_setup()

    return {
        "A_x": _A_in["x"],
        "A_c_kv": _A_in["c_kv"],
        "A_w_q": _A_in["w_q"],
        "A_w_uk": _A_in["w_uk"],
        "A_w_uv": _A_in["w_uv"],
        "A_w_o": _A_in["w_o"],
        "B_x": _B_in["x"],
        "B_Lambda_re": _B_in["Lambda_re"],
        "B_Lambda_im": _B_in["Lambda_im"],
        "B_B_re": _B_in["B_re"],
        "B_B_im": _B_in["B_im"],
        "B_C_re": _B_in["C_re"],
        "B_C_im": _B_in["C_im"],
        "B_log_dt": _B_in["log_dt"],
        "B_Dskip": _B_in["Dskip"],
        "gate_w": _w((lambda *s: _rng.normal(s) * 0.05)(448)),
    }

def reference(A_x, A_c_kv, A_w_q, A_w_uk, A_w_uv, A_w_o, B_x, B_Lambda_re, B_Lambda_im, B_B_re, B_B_im, B_C_re, B_C_im, B_log_dt, B_Dskip, gate_w):
    def _A_ref(x, c_kv, w_q, w_uk, w_uv, w_o):
        B, Sq, M = x.shape[0], x.shape[1], x.shape[2]
        Sk = c_kv.shape[1]
        H, D = w_q.shape[1], w_q.shape[2]
        q = jnp.einsum("bqm,mhd->bhqd", x, w_q)
        k = jnp.einsum("bkc,chd->bhkd", c_kv, w_uk)
        v = jnp.einsum("bkc,chd->bhkd", c_kv, w_uv)
        scores = jnp.einsum("bhqd,bhkd->bhqk", q, k) * (D ** -0.5)
        off = Sk - Sq
        qi = jnp.arange(Sq)[:, None]
        kj = jnp.arange(Sk)[None, :]
        cmask = kj <= (qi + off)
        scores = jnp.where(cmask[None, None], scores, -1e9)
        p = _softmax(scores, axis=-1)
        ctx = jnp.einsum("bhqk,bhkd->bhqd", p, v)
        return jnp.einsum("bhqd,hdm->bqm", ctx, w_o)

    def _B_ref(x, Lambda_re, Lambda_im, B_re, B_im, C_re, C_im, log_dt, Dskip):
        Bsz, L, H = x.shape
        Lam = Lambda_re + 1j * Lambda_im
        Bmat = B_re + 1j * B_im
        Cmat = C_re + 1j * C_im
        dt = jnp.exp(log_dt)
        Lam_bar = jnp.exp(dt * Lam)
        B_bar = ((Lam_bar - 1.0) / Lam)[:, None] * Bmat
        Bu = jnp.einsum("bld,pd->blp", x + 0j, B_bar)
        h = jnp.zeros_like(Bu[:, 0, :])
        hs = []
        for t in range(L):
            h = Lam_bar[None, :] * h + Bu[:, t, :]
            hs.append(h)
        hseq = jnp.stack(hs, 1)
        y = 2.0 * jnp.einsum("blp,dp->bld", hseq, Cmat).real + x * Dskip[None, None, :]
        return y

    x = A_x
    g = _sigmoid((x * gate_w).sum(-1, keepdims=True))
    a = _A_ref(x, A_c_kv, A_w_q, A_w_uk, A_w_uv, A_w_o)
    b = _B_ref(x, B_Lambda_re, B_Lambda_im, B_B_re, B_B_im, B_C_re, B_C_im, B_log_dt, B_Dskip)
    return g * a + (1 - g) * b
```

```python
import math

import jax
import jax.numpy as jnp
import jax.experimental.pallas as pl
import jax.experimental.pallas.tpu as pltpu

F32 = jnp.float32
BF16 = jnp.bfloat16
NT = (((1,), (1,)), ((), ()))

BQ = 256
SSM_T = 256


def _dot(a, b):
    return jnp.dot(a, b, preferred_element_type=F32)


def _dot_nt(a, b):
    return jax.lax.dot_general(a, b, NT, preferred_element_type=F32)


def _cmul(ar, ai, br, bi):
    return ar * br - ai * bi, ar * bi + ai * br


def _kernel(x_ref, bre_ref, bim_ref, cre_ref, cim_ref,
            lre_ref, lim_ref, ldt_ref, dsk_ref, gw_ref,
            ckv_hbm, wq_hbm, wuk_hbm, wuv_hbm, wo_hbm,
            out_ref,
            ckv, wq, wuk, wuv, wo, acc, q_s, k_s, v_s, sems):
    S, M = x_ref.shape
    H, D, _ = wo_hbm.shape

    wq32 = wq_hbm.bitcast(jnp.uint32)
    wuk32 = wuk_hbm.bitcast(jnp.uint32)
    wuv32 = wuv_hbm.bitcast(jnp.uint32)

    def pair_copies(hp, slot):
        return (
            pltpu.make_async_copy(wq32.at[:, hp, :], wq.at[slot], sems.at[1, slot]),
            pltpu.make_async_copy(wuk32.at[:, hp, :], wuk.at[slot], sems.at[2, slot]),
            pltpu.make_async_copy(wuv32.at[:, hp, :], wuv.at[slot], sems.at[3, slot]),
            pltpu.make_async_copy(wo_hbm.at[pl.ds(2 * hp, 2)], wo.at[slot], sems.at[4, slot]),
        )

    ckv_copy = pltpu.make_async_copy(ckv_hbm, ckv, sems.at[0, 0])
    ckv_copy.start()
    for cp in pair_copies(0, 0):
        cp.start()

    lre = lre_ref[...].astype(F32)
    lim = lim_ref[...].astype(F32)
    dt = jnp.exp(ldt_ref[...].astype(F32)).astype(BF16).astype(F32)
    mag = jnp.exp(dt * lre)
    a1 = (mag * jnp.cos(dt * lim), mag * jnp.sin(dt * lim))
    den = lre * lre + lim * lim
    nr, ni = a1[0] - 1.0, a1[1]
    coef = ((nr * lre + ni * lim) / den, (ni * lre - nr * lim) / den)
    a2 = _cmul(*a1, *a1)
    a4 = _cmul(*a2, *a2)
    a8 = _cmul(*a4, *a4)
    bc = lambda t: tuple(jnp.broadcast_to(z, (8, M)) for z in t)
    a8b = bc(a8)
    dsk = dsk_ref[...].astype(F32)
    gw = gw_ref[...].astype(F32)

    def ssm_chunk(c, carry):
        tail_r, tail_i, hr, hi = carry
        r0 = pl.multiple_of(c * SSM_T, SSM_T)
        xb = x_ref[pl.ds(r0, SSM_T), :]
        ur, ui = _cmul(_dot_nt(xb, bre_ref[...]), _dot_nt(xb, bim_ref[...]), *coef)
        yr = jnp.concatenate([tail_r, ur], axis=0)
        yi = jnp.concatenate([tail_i, ui], axis=0)
        for sh, a in ((1, a1), (2, a2), (4, a4)):
            dr, di = _cmul(pltpu.roll(yr, sh, 0), pltpu.roll(yi, sh, 0), *a)
            yr, yi = yr + dr, yi + di
        hs_r, hs_i = [], []
        for j in range(SSM_T // 8):
            pr, pi = _cmul(hr, hi, *a8b)
            hr = pr + yr[8 * (j + 1):8 * (j + 2)]
            hi = pi + yi[8 * (j + 1):8 * (j + 2)]
            hs_r.append(hr)
            hs_i.append(hi)
        h_r = jnp.concatenate(hs_r, axis=0).astype(BF16)
        h_i = jnp.concatenate(hs_i, axis=0).astype(BF16)
        xf = xb.astype(F32)
        y = 2.0 * (_dot_nt(h_r, cre_ref[...]) - _dot_nt(h_i, cim_ref[...])) + xf * dsk
        g = jax.nn.sigmoid(jnp.sum(xf * gw, axis=-1, keepdims=True))
        out_ref[pl.ds(r0, SSM_T), :] = (1.0 - g) * y
        return ur[SSM_T - 8:], ui[SSM_T - 8:], hr, hi

    z8 = jnp.zeros((8, M), F32)
    jax.lax.fori_loop(0, S // SSM_T, ssm_chunk, (z8, z8, z8, z8))

    acc[...] = jnp.zeros(acc.shape, F32)
    ckv_copy.wait()

    qscale = (D ** -0.5) * math.log2(math.e)

    def unpack(words, odd):
        sh = (16 * (1 - odd)).astype(jnp.uint32)
        return pltpu.bitcast((words << sh) & jnp.uint32(0xFFFF0000), F32).astype(BF16)

    def head(h, _):
        hp = h // 2
        odd = h % 2
        slot = hp % 2

        @pl.when(odd == 0)
        def _():
            @pl.when(hp + 1 < H // 2)
            def _():
                for cp in pair_copies(hp + 1, 1 - slot):
                    cp.start()
            for cp in pair_copies(hp, slot):
                cp.wait()

        q_s[...] = (_dot(x_ref[...], unpack(wq[slot], odd)) * qscale).astype(BF16)
        k_s[...] = _dot(ckv[...], unpack(wuk[slot], odd)).astype(BF16)
        v_s[...] = _dot(ckv[...], unpack(wuv[slot], odd)).astype(BF16)
        w_out = wo[slot, odd]

        row = jax.lax.broadcasted_iota(jnp.int32, (BQ, BQ), 0)
        col = jax.lax.broadcasted_iota(jnp.int32, (BQ, BQ), 1)
        causal = col <= row
        for i in range(S // BQ):
            lo, hi = i * BQ, (i + 1) * BQ
            qb = q_s[lo:hi, :]
            s = jnp.where(causal, _dot_nt(qb, k_s[lo:hi, :]), -1e9)
            if i > 0:
                s = jnp.concatenate([_dot_nt(qb, k_s[0:lo, :]), s], axis=1)
            m = jnp.max(s, axis=-1, keepdims=True)
            p = jnp.exp2(s - m)
            l = jnp.sum(p, axis=-1, keepdims=True)
            ctx = _dot(p.astype(BF16), v_s[0:hi, :]) * (1.0 / l)
            acc[lo:hi, :] += _dot(ctx.astype(BF16), w_out)
        return 0

    jax.lax.fori_loop(0, H, head, 0)

    xf = x_ref[...].astype(F32)
    g = jax.nn.sigmoid(jnp.sum(xf * gw, axis=-1, keepdims=True))
    out_ref[...] = out_ref[...] + g * acc[...]


@jax.jit
def pallas_gated_mix__compressed_kv_cla__ssm_conv_s5__prompt_kernel(
    A_x: jax.Array,
    A_c_kv: jax.Array,
    A_w_q: jax.Array,
    A_w_uk: jax.Array,
    A_w_uv: jax.Array,
    A_w_o: jax.Array,
    B_x: jax.Array,
    B_Lambda_re: jax.Array,
    B_Lambda_im: jax.Array,
    B_B_re: jax.Array,
    B_B_im: jax.Array,
    B_C_re: jax.Array,
    B_C_im: jax.Array,
    B_log_dt: jax.Array,
    B_Dskip: jax.Array,
    gate_w: jax.Array,
):
    del B_x
    B, S, M = A_x.shape
    Dc, H, D = A_w_uk.shape
    assert B == 1 and A_c_kv.shape[1] == S
    row = lambda v: v.reshape(1, -1)
    vmem = pl.BlockSpec(memory_space=pltpu.VMEM)
    hbm = pl.BlockSpec(memory_space=pl.ANY)
    out = pl.pallas_call(
        _kernel,
        in_specs=[vmem] * 10 + [hbm] * 5,
        out_specs=vmem,
        out_shape=jax.ShapeDtypeStruct((S, M), F32),
        scratch_shapes=[
            pltpu.VMEM((S, Dc), BF16),
            pltpu.VMEM((2, M, D), jnp.uint32),
            pltpu.VMEM((2, Dc, D), jnp.uint32),
            pltpu.VMEM((2, Dc, D), jnp.uint32),
            pltpu.VMEM((2, 2, D, M), BF16),
            pltpu.VMEM((S, M), F32),
            pltpu.VMEM((S, D), BF16),
            pltpu.VMEM((S, D), BF16),
            pltpu.VMEM((S, D), BF16),
            pltpu.SemaphoreType.DMA((5, 2)),
        ],
        compiler_params=pltpu.CompilerParams(vmem_limit_bytes=100 * 2**20),
    )(A_x.reshape(S, M), B_B_re, B_B_im, B_C_re, B_C_im,
      row(B_Lambda_re), row(B_Lambda_im), row(B_log_dt), row(B_Dskip), row(gate_w),
      A_c_kv.reshape(S, Dc), A_w_q, A_w_uk, A_w_uv, A_w_o)
    return out.reshape(B, S, M)
```

```python
import math

import jax
import jax.numpy as jnp
import jax.experimental.pallas as pl
import jax.experimental.pallas.tpu as pltpu

F32 = jnp.float32
BF16 = jnp.bfloat16
LANES = 128

BQ = 256
SSM_T = 256


def _dot(a, b, ca=1, cb=0):
    return jax.lax.dot_general(a, b, (((ca,), (cb,)), ((), ())), preferred_element_type=F32)


def _cmul(ar, ai, br, bi):
    return ar * br - ai * bi, ar * bi + ai * br


def _kernel(lre_ref, lim_ref, ldt_ref, dsk_ref, gw_ref,
            xt_hbm, bre_hbm, bim_hbm, cre_hbm, cim_hbm,
            ckv_hbm, wq_hbm, wuk_hbm, wuv_hbm, wot_hbm,
            out_hbm,
            xt, bcat, cre, cim, ccat, ckv, wq, wuk, wuv, wot, acc, g_s, qt_s, k_s, vt_s,
            sems, wsems):
    M, S = xt.shape
    H, _, D = wot_hbm.shape
    PM = M // LANES * LANES
    PR = M - PM
    assert 2 * PR == LANES

    def copy(src, dst, i):
        return pltpu.make_async_copy(src, dst, sems.at[i])

    first = [
        copy(xt_hbm.at[:, pl.ds(0, SSM_T)], xt.at[:, pl.ds(0, SSM_T)], 0),
        copy(bre_hbm.at[pl.ds(0, PM)], bcat.at[pl.ds(0, PM)], 1),
        copy(bim_hbm.at[pl.ds(0, PM)], bcat.at[pl.ds(PM, PM)], 2),
        copy(bre_hbm.at[pl.ds(PM, PR)], bcat.at[pl.ds(2 * PM, PR)], 3),
        copy(bim_hbm.at[pl.ds(PM, PR)], bcat.at[pl.ds(2 * PM + PR, PR)], 4),
        copy(cre_hbm, cre, 5),
        copy(cim_hbm, cim, 6),
    ]
    x_rest = copy(xt_hbm.at[:, pl.ds(SSM_T, S - SSM_T)], xt.at[:, pl.ds(SSM_T, S - SSM_T)], 7)
    ckv_copy = copy(ckv_hbm, ckv, 8)

    wq32 = wq_hbm.bitcast(jnp.uint32)
    wuk32 = wuk_hbm.bitcast(jnp.uint32)
    wuv32 = wuv_hbm.bitcast(jnp.uint32)

    def pair_copies(hp, slot):
        return (
            pltpu.make_async_copy(wq32.at[:, hp, :], wq.at[slot], wsems.at[0, slot]),
            pltpu.make_async_copy(wuk32.at[:, hp, :], wuk.at[slot], wsems.at[1, slot]),
            pltpu.make_async_copy(wuv32.at[:, hp, :], wuv.at[slot], wsems.at[2, slot]),
            pltpu.make_async_copy(wot_hbm.at[pl.ds(2 * hp, 2)], wot.at[slot], wsems.at[3, slot]),
        )

    for cp in first:
        cp.start()
    x_rest.start()

    def row(ref):
        v = ref[...].astype(F32).reshape(1, M)
        return jnp.concatenate([v, v[:, PM:]], axis=1)

    def column(ref):
        return jnp.broadcast_to(row(ref), (LANES, PM + LANES)).T[:M]

    lre, lim = row(lre_ref), row(lim_ref)
    dt = jnp.exp(row(ldt_ref)).astype(BF16).astype(F32)
    mag = jnp.exp(dt * lre)
    ar, ai = mag * jnp.cos(dt * lim), mag * jnp.sin(dt * lim)
    den = lre * lre + lim * lim
    cr = 2.0 * ((ar - 1.0) * lre + ai * lim) / den
    ci = 2.0 * (ai * lre - (ar - 1.0) * lim) / den
    a1 = (ar, -ai)
    a2 = _cmul(*a1, *a1)
    a4 = _cmul(*a2, *a2)
    a8 = tuple(jnp.broadcast_to(z, (8, PM + LANES)) for z in _cmul(*a4, *a4))
    dsk = jnp.tile(column(dsk_ref), (1, SSM_T // LANES))
    gw = jnp.tile(column(gw_ref), (1, SSM_T // LANES))

    for cp in first:
        cp.wait()
    ckv_copy.start()
    for cp in pair_copies(0, 0):
        cp.start()

    ccat[:, 0:PM] = cre[:, 0:PM]
    ccat[:, PM:2 * PM] = cim[:, 0:PM]
    ccat[:, 2 * PM:] = jnp.concatenate([cre[:, PM:], cim[:, PM:]], axis=1)

    low_half = jax.lax.broadcasted_iota(jnp.int32, (SSM_T, LANES), 1) < PR
    tail_r = tail_i = hr = hi = jnp.zeros((8, PM + LANES), F32)
    for c in range(S // SSM_T):
        cols = slice(c * SSM_T, (c + 1) * SSM_T)
        if c == 1:
            x_rest.wait()
        xb = xt[:, cols]
        b = _dot(xb, bcat[...], 0, 1)
        bt = b[:, 2 * PM:]
        br = jnp.concatenate([b[:, :PM], bt], axis=1)
        bi = jnp.concatenate([b[:, PM:2 * PM], pltpu.roll(bt, PR, 1)], axis=1)
        ur, ui = cr * br - ci * bi, -(cr * bi + ci * br)
        yr = jnp.concatenate([tail_r, ur], axis=0)
        yi = jnp.concatenate([tail_i, ui], axis=0)
        tail_r, tail_i = ur[SSM_T - 8:], ui[SSM_T - 8:]
        for sh, a in ((1, a1), (2, a2), (4, a4)):
            dr, di = _cmul(pltpu.roll(yr, sh, 0), pltpu.roll(yi, sh, 0), *a)
            yr, yi = yr + dr, yi + di
        hs_r, hs_i = [], []
        for j in range(1, SSM_T // 8 + 1):
            pr, pi = _cmul(hr, hi, *a8)
            hr = pr + yr[8 * j:8 * j + 8]
            hi = pi + yi[8 * j:8 * j + 8]
            hs_r.append(hr)
            hs_i.append(hi)
        h_r = jnp.concatenate(hs_r, axis=0)
        h_i = jnp.concatenate(hs_i, axis=0)
        h_t = jnp.where(low_half, h_r[:, PM:], pltpu.roll(h_i[:, PM:], PR, 1))
        hcat = jnp.concatenate([h_r[:, :PM], h_i[:, :PM], h_t], axis=1).astype(BF16)
        xf = xb.astype(F32)
        y = _dot(ccat[...], hcat, 1, 1) + xf * dsk
        g = jax.nn.sigmoid(jnp.sum(xf * gw, axis=0, keepdims=True))
        g_s[:, cols] = g
        acc[:, cols] = (1.0 - g) * y

    ckv_copy.wait()

    qscale = (D ** -0.5) * math.log2(math.e)

    def unpack(words, odd):
        sh = (16 * (1 - odd)).astype(jnp.uint32)
        return pltpu.bitcast((words << sh) & jnp.uint32(0xFFFF0000), F32).astype(BF16)

    def head(h, _):
        hp = h // 2
        odd = h % 2
        slot = hp % 2

        @pl.when(odd == 0)
        def _():
            @pl.when(hp + 1 < H // 2)
            def _():
                for cp in pair_copies(hp + 1, 1 - slot):
                    cp.start()
            for cp in pair_copies(hp, slot):
                cp.wait()

        k_s[...] = _dot(ckv[...], unpack(wuk[slot], odd)).astype(BF16)
        qt_s[...] = (_dot(unpack(wq[slot], odd), xt[...], 0, 0) * qscale).astype(BF16)
        vt_s[...] = _dot(unpack(wuv[slot], odd), ckv[...], 0, 1).astype(BF16)
        w_out = wot[slot, odd]

        kj = jax.lax.broadcasted_iota(jnp.int32, (LANES, LANES), 0)
        qi = jax.lax.broadcasted_iota(jnp.int32, (LANES, LANES), 1)
        causal = kj <= qi
        for i in range(S // BQ):
            ctx = []
            for t in range(i * BQ // LANES, (i + 1) * BQ // LANES):
                lo, hi = t * LANES, (t + 1) * LANES
                s = _dot(k_s[0:hi, :], qt_s[:, lo:hi])
                sd = jnp.where(causal, s[lo:hi], -1e9)
                s = jnp.concatenate([s[0:lo], sd], axis=0) if lo else sd
                m = jnp.max(s, axis=0, keepdims=True)
                p = jnp.exp2(s - m)
                l = jnp.sum(p, axis=0, keepdims=True)
                ctx.append((_dot(vt_s[:, 0:hi], p.astype(BF16)) * (g_s[:, lo:hi] / l)).astype(BF16))
            acc[:, i * BQ:(i + 1) * BQ] += _dot(w_out, jnp.concatenate(ctx, axis=1))
        return 0

    jax.lax.fori_loop(0, H, head, 0)

    out_copy = copy(acc, out_hbm, 0)
    out_copy.start()
    out_copy.wait()


@jax.jit
def pallas_gated_mix__compressed_kv_cla__ssm_conv_s5__prompt_kernel(
    A_x: jax.Array,
    A_c_kv: jax.Array,
    A_w_q: jax.Array,
    A_w_uk: jax.Array,
    A_w_uv: jax.Array,
    A_w_o: jax.Array,
    B_x: jax.Array,
    B_Lambda_re: jax.Array,
    B_Lambda_im: jax.Array,
    B_B_re: jax.Array,
    B_B_im: jax.Array,
    B_C_re: jax.Array,
    B_C_im: jax.Array,
    B_log_dt: jax.Array,
    B_Dskip: jax.Array,
    gate_w: jax.Array,
):
    del B_x
    B, S, M = A_x.shape
    Dc, H, D = A_w_uk.shape
    assert B == 1 and A_c_kv.shape[1] == S
    vmem = pl.BlockSpec(memory_space=pltpu.VMEM)
    hbm = pl.BlockSpec(memory_space=pltpu.HBM)
    out_t = pl.pallas_call(
        _kernel,
        in_specs=[vmem] * 5 + [hbm] * 10,
        out_specs=hbm,
        out_shape=pltpu.HBM((M, S), F32),
        scratch_shapes=[
            pltpu.VMEM((M, S), BF16),
            pltpu.VMEM((2 * M, M), BF16),
            pltpu.VMEM((M, M), BF16),
            pltpu.VMEM((M, M), BF16),
            pltpu.VMEM((M, 2 * M), BF16),
            pltpu.VMEM((S, Dc), BF16),
            pltpu.VMEM((2, M, D), jnp.uint32),
            pltpu.VMEM((2, Dc, D), jnp.uint32),
            pltpu.VMEM((2, Dc, D), jnp.uint32),
            pltpu.VMEM((2, 2, M, D), BF16),
            pltpu.VMEM((M, S), F32),
            pltpu.VMEM((1, S), F32),
            pltpu.VMEM((D, S), BF16),
            pltpu.VMEM((S, D), BF16),
            pltpu.VMEM((D, S), BF16),
            pltpu.SemaphoreType.DMA((9,)),
            pltpu.SemaphoreType.DMA((4, 2)),
        ],
        compiler_params=pltpu.CompilerParams(vmem_limit_bytes=64 * 2**20),
    )(B_Lambda_re, B_Lambda_im, B_log_dt, B_Dskip, gate_w,
      A_x.reshape(S, M).T, B_B_re, B_B_im, B_C_re, B_C_im,
      A_c_kv.reshape(S, Dc), A_w_q, A_w_uk, A_w_uv, A_w_o.transpose(0, 2, 1))
    return out_t.T.reshape(B, S, M)
```

```python
import functools
import math

import jax
import jax.numpy as jnp
import jax.experimental.pallas as pl
import jax.experimental.pallas.tpu as pltpu

F32 = jnp.float32
BF16 = jnp.bfloat16
LANES = 128

BQ = 256
QT=128
DESC=0
SK1=1
SK2=2
SK3=3
PK=512
PV=256
PQ=512
C0=3
SSM_T = 256


def _dot(a, b, ca=1, cb=0):
    return jax.lax.dot_general(a, b, (((ca,), (cb,)), ((), ())), preferred_element_type=F32)


def _cmul(ar, ai, br, bi):
    return ar * br - ai * bi, ar * bi + ai * br


def _kernel(lre_ref, lim_ref, ldt_ref, dsk_ref, gw_ref,
            xt_hbm, bre_hbm, bim_hbm, cre_hbm, cim_hbm,
            ckv_hbm, wq_hbm, wuk_hbm, wuv_hbm, wot_hbm,
            out_hbm,
            xt, bcat, cre, cim, ccat, ckv, wq, wuk, wuv, wot, acc, g_s, qt_s, k_s, vt_s,
            wk_b, wq_b, wv_b, sems, wsems, osems):
    M, S = xt.shape
    H, _, D = wot_hbm.shape
    PM = M // LANES * LANES
    PR = M - PM
    assert 2 * PR == LANES

    def copy(src, dst, i):
        return pltpu.make_async_copy(src, dst, sems.at[i])

    first = [
        copy(xt_hbm.at[:, pl.ds(0, SSM_T)], xt.at[:, pl.ds(0, SSM_T)], 0),
        copy(bre_hbm.at[pl.ds(0, PM)], bcat.at[pl.ds(0, PM)], 1),
        copy(bim_hbm.at[pl.ds(0, PM)], bcat.at[pl.ds(PM, PM)], 2),
        copy(bre_hbm.at[pl.ds(PM, PR)], bcat.at[pl.ds(2 * PM, PR)], 3),
        copy(bim_hbm.at[pl.ds(PM, PR)], bcat.at[pl.ds(2 * PM + PR, PR)], 4),
        copy(cre_hbm, cre, 5),
        copy(cim_hbm, cim, 6),
    ]
    x_rest = copy(xt_hbm.at[:, pl.ds(SSM_T, S - SSM_T)], xt.at[:, pl.ds(SSM_T, S - SSM_T)], 7)
    ckv_copy = copy(ckv_hbm, ckv, 8)

    wq32 = wq_hbm.bitcast(jnp.uint32)
    wuk32 = wuk_hbm.bitcast(jnp.uint32)
    wuv32 = wuv_hbm.bitcast(jnp.uint32)

    def pair_copies(hp, slot):
        return (
            pltpu.make_async_copy(wq32.at[:, hp, :], wq.at[slot], wsems.at[0, slot]),
            pltpu.make_async_copy(wuk32.at[:, hp, :], wuk.at[slot], wsems.at[1, slot]),
            pltpu.make_async_copy(wuv32.at[:, hp, :], wuv.at[slot], wsems.at[2, slot]),
        )

    def wo_copy(h):
        return pltpu.make_async_copy(wot_hbm.at[h], wot.at[h % 2], wsems.at[3, h % 2])

    qscale = (D ** -0.5) * math.log2(math.e)

    def project(h):
        slot, wslot = h % 2, (h // 2) % 2
        sh = jnp.uint32(16) * jnp.asarray(1 - h % 2).astype(jnp.uint32)

        def unpack(ref):
            return pltpu.bitcast((ref[wslot] << sh) & jnp.uint32(0xFFFF0000), F32)

        def prep_k():
            wk_b[...] = unpack(wuk).astype(BF16)

        def prep_q():
            wq_b[...] = unpack(wq).astype(BF16)

        def prep_v():
            wv_b[...] = unpack(wuv).astype(BF16).T

        def k(r):
            k_s[slot, r, :] = _dot(ckv[r, :], wk_b[...]).astype(BF16)

        def q(r):
            qt_s[slot, :, r] = (_dot(wq_b[...], xt[:, r], 0, 0) * qscale).astype(BF16)

        def v(r):
            vt_s[slot, :, r] = _dot(wv_b[...], ckv[r, :], 1, 1).astype(BF16)

        part = lambda n: [slice(i, i + n) for i in range(0, S, n)]
        return ([prep_k] + [functools.partial(k, r) for r in part(PK)] + [prep_v, prep_q]
                + [functools.partial(v, r) for r in part(PV)]
                + [functools.partial(q, r) for r in part(PQ)])

    def spread(steps, weights):
        out, done, cum = [], 0, 0
        for w in weights:
            cum += w
            upto = round(len(steps) * cum / sum(weights))
            out.append(steps[done:upto])
            done = upto
        return out

    for cp in first:
        cp.start()
    x_rest.start()

    def row(ref):
        v = ref[...].astype(F32).reshape(1, M)
        return jnp.concatenate([v, v[:, PM:]], axis=1)

    def column(ref):
        return jnp.broadcast_to(row(ref), (LANES, PM + LANES)).T[:M]

    lre, lim = row(lre_ref), row(lim_ref)
    dt = jnp.exp(row(ldt_ref)).astype(BF16).astype(F32)
    mag = jnp.exp(dt * lre)
    ar, ai = mag * jnp.cos(dt * lim), mag * jnp.sin(dt * lim)
    den = lre * lre + lim * lim
    cr = 2.0 * ((ar - 1.0) * lre + ai * lim) / den
    ci = 2.0 * (ai * lre - (ar - 1.0) * lim) / den
    a1 = (ar, -ai)
    a2 = _cmul(*a1, *a1)
    a4 = _cmul(*a2, *a2)
    a8 = tuple(jnp.broadcast_to(z, (8, PM + LANES)) for z in _cmul(*a4, *a4))
    dsk = jnp.tile(column(dsk_ref), (1, SSM_T // LANES))
    gw = jnp.tile(column(gw_ref), (1, SSM_T // LANES))

    for cp in first:
        cp.wait()
    ckv_copy.start()
    for cp in pair_copies(0, 0):
        cp.start()
    wo_copy(0).start()

    ccat[:, 0:PM] = cre[:, 0:PM]
    ccat[:, PM:2 * PM] = cim[:, 0:PM]
    ccat[:, 2 * PM:] = jnp.concatenate([cre[:, PM:], cim[:, PM:]], axis=1)

    low_half = jax.lax.broadcasted_iota(jnp.int32, (SSM_T, LANES), 1) < PR
    tail_r = tail_i = hr = hi = jnp.zeros((8, PM + LANES), F32)
    nc = S // SSM_T
    fill = spread(project(0), [0] * C0 + [1] * (nc - C0))
    for c in range(nc):
        if c == C0:
            ckv_copy.wait()
            for cp in pair_copies(0, 0):
                cp.wait()
            for cp in pair_copies(1, 1):
                cp.start()
        cols = slice(c * SSM_T, (c + 1) * SSM_T)
        if c == 1:
            x_rest.wait()
        xb = xt[:, cols]
        b = _dot(xb, bcat[...], 0, 1)
        bt = b[:, 2 * PM:]
        br = jnp.concatenate([b[:, :PM], bt], axis=1)
        bi = jnp.concatenate([b[:, PM:2 * PM], pltpu.roll(bt, PR, 1)], axis=1)
        ur, ui = cr * br - ci * bi, -(cr * bi + ci * br)
        yr = jnp.concatenate([tail_r, ur], axis=0)
        yi = jnp.concatenate([tail_i, ui], axis=0)
        tail_r, tail_i = ur[SSM_T - 8:], ui[SSM_T - 8:]
        for sh, a in ((1, a1), (2, a2), (4, a4)):
            dr, di = _cmul(pltpu.roll(yr, sh, 0), pltpu.roll(yi, sh, 0), *a)
            yr, yi = yr + dr, yi + di
        for f in fill[c]:
            f()
        hs_r, hs_i = [], []
        for j in range(1, SSM_T // 8 + 1):
            pr, pi = _cmul(hr, hi, *a8)
            hr = pr + yr[8 * j:8 * j + 8]
            hi = pi + yi[8 * j:8 * j + 8]
            hs_r.append(hr)
            hs_i.append(hi)
        h_r = jnp.concatenate(hs_r, axis=0)
        h_i = jnp.concatenate(hs_i, axis=0)
        h_t = jnp.where(low_half, h_r[:, PM:], pltpu.roll(h_i[:, PM:], PR, 1))
        hcat = jnp.concatenate([h_r[:, :PM], h_i[:, :PM], h_t], axis=1).astype(BF16)
        xf = xb.astype(F32)
        y = _dot(ccat[...], hcat, 1, 1) + xf * dsk
        g = jax.nn.sigmoid(jnp.sum(xf * gw, axis=0, keepdims=True))
        g_s[:, cols] = g
        acc[:, cols] = (1.0 - g) * y

    def attend(h, fill, block_done):
        slot = h % 2
        kj = jax.lax.broadcasted_iota(jnp.int32, (QT, QT), 0)
        qi = jax.lax.broadcasted_iota(jnp.int32, (QT, QT), 1)
        causal = kj <= qi

        def scores(t):
            lo, hi = t * QT, (t + 1) * QT
            s = _dot(k_s[slot, 0:hi, :], qt_s[slot, :, lo:hi])
            sd = jnp.where(causal, s[lo:hi], -1e9)
            return jnp.concatenate([s[0:lo], sd], axis=0) if lo else sd

        def softmax(s):
            p = jnp.exp2(s - jnp.max(s, axis=0, keepdims=True))
            return p.astype(BF16), jnp.sum(p, axis=0, keepdims=True)

        def context(t, p, l):
            lo, hi = t * QT, (t + 1) * QT
            return (_dot(vt_s[slot, :, 0:hi], p) * (g_s[:, lo:hi] / l)).astype(BF16)

        n = S // QT
        per = BQ // QT
        order = list(range(n))
        if DESC:
            order = order[::-1]
        steps = n + SK3
        fill = spread(fill, [0] * SK1 + [order[i] + 1 for i in range(n)] + [0] * (SK3 - SK1))
        s_q, p_q, ctx = {}, {}, {}
        for step in range(steps):
            if step < n:
                s_q[order[step]] = scores(order[step])
            for f in fill[step]:
                f()
            if 0 <= step - SK1 < n:
                t = order[step - SK1]
                p_q[t] = softmax(s_q.pop(t))
            if 0 <= step - SK2 < n:
                t = order[step - SK2]
                ctx[t] = context(t, *p_q.pop(t))
            if 0 <= step - SK3 < n:
                i = order[step - SK3] // per
                ts = range(i * per, (i + 1) * per)
                if order[step - SK3] == (ts[0] if DESC else ts[-1]):
                    c = jnp.concatenate([ctx.pop(t) for t in ts], axis=1)
                    acc[:, i * BQ:(i + 1) * BQ] += _dot(wot[slot], c)
                    block_done(i)

    def head(h, _):
        @pl.when(h % 2 == 1)
        def _():
            hp = (h + 1) // 2
            for cp in pair_copies(hp, hp % 2):
                cp.wait()

            @pl.when(hp + 1 < H // 2)
            def _():
                for cp in pair_copies(hp + 1, 1 - hp % 2):
                    cp.start()

        wo_copy(h).wait()
        wo_copy(h + 1).start()
        attend(h, project(h + 1), lambda i: None)
        return 0

    jax.lax.fori_loop(0, H - 1, head, 0)

    def out_copy(i):
        cols = pl.ds(i * BQ, BQ)
        return pltpu.make_async_copy(acc.at[:, cols], out_hbm.at[:, cols], osems.at[i])

    wo_copy(H - 1).wait()
    attend(H - 1, [], lambda i: out_copy(i).start())
    for i in range(S // BQ):
        out_copy(i).wait()


@jax.jit
def pallas_gated_mix__compressed_kv_cla__ssm_conv_s5__prompt_kernel(
    A_x: jax.Array,
    A_c_kv: jax.Array,
    A_w_q: jax.Array,
    A_w_uk: jax.Array,
    A_w_uv: jax.Array,
    A_w_o: jax.Array,
    B_x: jax.Array,
    B_Lambda_re: jax.Array,
    B_Lambda_im: jax.Array,
    B_B_re: jax.Array,
    B_B_im: jax.Array,
    B_C_re: jax.Array,
    B_C_im: jax.Array,
    B_log_dt: jax.Array,
    B_Dskip: jax.Array,
    gate_w: jax.Array,
):
    del B_x
    B, S, M = A_x.shape
    Dc, H, D = A_w_uk.shape
    assert B == 1 and A_c_kv.shape[1] == S
    vmem = pl.BlockSpec(memory_space=pltpu.VMEM)
    hbm = pl.BlockSpec(memory_space=pltpu.HBM)
    out_t = pl.pallas_call(
        _kernel,
        in_specs=[vmem] * 5 + [hbm] * 10,
        out_specs=hbm,
        out_shape=pltpu.HBM((M, S), F32),
        scratch_shapes=[
            pltpu.VMEM((M, S), BF16),
            pltpu.VMEM((2 * M, M), BF16),
            pltpu.VMEM((M, M), BF16),
            pltpu.VMEM((M, M), BF16),
            pltpu.VMEM((M, 2 * M), BF16),
            pltpu.VMEM((S, Dc), BF16),
            pltpu.VMEM((2, M, D), jnp.uint32),
            pltpu.VMEM((2, Dc, D), jnp.uint32),
            pltpu.VMEM((2, Dc, D), jnp.uint32),
            pltpu.VMEM((2, M, D), BF16),
            pltpu.VMEM((M, S), F32),
            pltpu.VMEM((1, S), F32),
            pltpu.VMEM((2, D, S), BF16),
            pltpu.VMEM((2, S, D), BF16),
            pltpu.VMEM((2, D, S), BF16),
            pltpu.VMEM((Dc, D), BF16),
            pltpu.VMEM((M, D), BF16),
            pltpu.VMEM((D, Dc), BF16),
            pltpu.SemaphoreType.DMA((9,)),
            pltpu.SemaphoreType.DMA((4, 2)),
            pltpu.SemaphoreType.DMA((S // BQ,)),
        ],
        compiler_params=pltpu.CompilerParams(vmem_limit_bytes=64 * 2**20),
    )(B_Lambda_re, B_Lambda_im, B_log_dt, B_Dskip, gate_w,
      A_x.reshape(S, M).T, B_B_re, B_B_im, B_C_re, B_C_im,
      A_c_kv.reshape(S, Dc), A_w_q, A_w_uk, A_w_uv, A_w_o.transpose(0, 2, 1))
    return out_t.T.reshape(B, S, M)
```

```python
import functools
import math

import jax
import jax.numpy as jnp
import jax.experimental.pallas as pl
import jax.experimental.pallas.tpu as pltpu

F32 = jnp.float32
BF16 = jnp.bfloat16
LANES = 128
S_=2048

BQ = 512
QT=128
CK=512
OM=0
FR=32
FW=(1,1)
ORDER=list(range(S_//QT))
SK1=2
SK2=4
SK3=5
PK=512
PV=256
PQ=512
C0=3
SSM_T = 512


def _dot(a, b, ca=1, cb=0):
    return jax.lax.dot_general(a, b, (((ca,), (cb,)), ((), ())), preferred_element_type=F32)


def _cmul(ar, ai, br, bi):
    return ar * br - ai * bi, ar * bi + ai * br


def _kernel(lre_ref, lim_ref, ldt_ref, dsk_ref, gw_ref,
            xt_hbm, bre_hbm, bim_hbm, cre_hbm, cim_hbm,
            ckv_hbm, wq_hbm, wuk_hbm, wuv_hbm, wot_hbm,
            out_hbm,
            xt, bcat, cre, cim, ccat, ckv, wq, wuk, wuv, wot, acc, g_s, qt_s, k_s, vt_s,
            wk_b, wq_b, wv_b, sems, wsems, osems):
    M, S = xt.shape
    H, _, D = wot_hbm.shape
    PM = M // LANES * LANES
    PR = M - PM
    assert 2 * PR == LANES

    def copy(src, dst, i):
        return pltpu.make_async_copy(src, dst, sems.at[i])

    first = [
        copy(xt_hbm.at[:, pl.ds(0, SSM_T)], xt.at[:, pl.ds(0, SSM_T)], 0),
        copy(bre_hbm.at[pl.ds(0, PM)], bcat.at[pl.ds(0, PM)], 1),
        copy(bim_hbm.at[pl.ds(0, PM)], bcat.at[pl.ds(PM, PM)], 2),
        copy(bre_hbm.at[pl.ds(PM, PR)], bcat.at[pl.ds(2 * PM, PR)], 3),
        copy(bim_hbm.at[pl.ds(PM, PR)], bcat.at[pl.ds(2 * PM + PR, PR)], 4),
        copy(cre_hbm, cre, 5),
        copy(cim_hbm, cim, 6),
    ]
    x_rest = copy(xt_hbm.at[:, pl.ds(SSM_T, S - SSM_T)], xt.at[:, pl.ds(SSM_T, S - SSM_T)], 7)
    ckv_copy = copy(ckv_hbm, ckv, 8)

    wq32 = wq_hbm.bitcast(jnp.uint32)
    wuk32 = wuk_hbm.bitcast(jnp.uint32)
    wuv32 = wuv_hbm.bitcast(jnp.uint32)

    def pair_copies(hp, slot):
        return (
            pltpu.make_async_copy(wq32.at[:, hp, :], wq.at[slot], wsems.at[0, slot]),
            pltpu.make_async_copy(wuk32.at[:, hp, :], wuk.at[slot], wsems.at[1, slot]),
            pltpu.make_async_copy(wuv32.at[:, hp, :], wuv.at[slot], wsems.at[2, slot]),
        )

    def wo_copy(h):
        return pltpu.make_async_copy(wot_hbm.at[h], wot.at[h % 2], wsems.at[3, h % 2])

    qscale = (D ** -0.5) * math.log2(math.e)

    def project(h):
        slot, wslot = 0, (h // 2) % 2
        sh = jnp.uint32(16) * jnp.asarray(1 - h % 2).astype(jnp.uint32)

        def unpack(ref):
            return pltpu.bitcast((ref[wslot] << sh) & jnp.uint32(0xFFFF0000), F32)

        def prep_k():
            wk_b[...] = unpack(wuk).astype(BF16)

        def prep_q():
            wq_b[...] = unpack(wq).astype(BF16)

        def prep_v():
            wv_b[...] = unpack(wuv).astype(BF16).T

        def k(r):
            k_s[slot, r, :] = _dot(ckv[r, :], wk_b[...]).astype(BF16)

        def q(r):
            qt_s[slot, :, r] = (_dot(wq_b[...], xt[:, r], 0, 0) * qscale).astype(BF16)

        def v(r):
            vt_s[slot, :, r] = _dot(wv_b[...], ckv[r, :], 1, 1).astype(BF16)

        part = lambda n: [slice(i, i + n) for i in range(0, S, n)]
        return ([prep_k] + [functools.partial(k, r) for r in part(PK)] + [prep_v, prep_q]
                + [functools.partial(v, r) for r in part(PV)]
                + [functools.partial(q, r) for r in part(PQ)])

    def spread(steps, weights):
        out, done, cum = [], 0, 0
        for w in weights:
            cum += w
            upto = round(len(steps) * cum / sum(weights))
            out.append(steps[done:upto])
            done = upto
        return out

    def interleave(lanes):
        keyed = [((i + 0.5) / len(lane), j, f) for j, lane in enumerate(lanes) for i, f in enumerate(lane)]
        for _, _, f in sorted(keyed, key=lambda e: e[:2]):
            f()

    for cp in first:
        cp.start()
    x_rest.start()

    def row(ref):
        v = ref[...].astype(F32).reshape(1, M)
        return jnp.concatenate([v, v[:, PM:]], axis=1)

    def column(ref):
        return jnp.broadcast_to(row(ref), (LANES, PM + LANES)).T[:M]

    lre, lim = row(lre_ref), row(lim_ref)
    dt = jnp.exp(row(ldt_ref)).astype(BF16).astype(F32)
    mag = jnp.exp(dt * lre)
    ar, ai = mag * jnp.cos(dt * lim), mag * jnp.sin(dt * lim)
    den = lre * lre + lim * lim
    cr = 2.0 * ((ar - 1.0) * lre + ai * lim) / den
    ci = 2.0 * (ai * lre - (ar - 1.0) * lim) / den
    a1 = (ar, -ai)
    a2 = _cmul(*a1, *a1)
    a4 = _cmul(*a2, *a2)
    a8 = tuple(jnp.broadcast_to(z, (8, PM + LANES)) for z in _cmul(*a4, *a4))
    dsk = jnp.tile(column(dsk_ref), (1, SSM_T // LANES))
    gw = jnp.tile(column(gw_ref), (1, SSM_T // LANES))

    for cp in first:
        cp.wait()
    ckv_copy.start()
    for cp in pair_copies(0, 0):
        cp.start()
    wo_copy(0).start()

    ccat[:, 0:PM] = cre[:, 0:PM]
    ccat[:, PM:2 * PM] = cim[:, 0:PM]
    ccat[:, 2 * PM:] = jnp.concatenate([cre[:, PM:], cim[:, PM:]], axis=1)

    low_half = jax.lax.broadcasted_iota(jnp.int32, (SSM_T, LANES), 1) < PR
    nc, nt = S // SSM_T, PM // LANES + 1
    zero = jnp.zeros((8, LANES), F32)
    tail, state = [(zero, zero)] * nt, [(zero, zero)] * nt
    b_q, y_q, h_q = {}, {}, {}
    tile = lambda v, j: v[:, j * LANES:(j + 1) * LANES]

    def ssm_in(c, j):
        xb = xt[:, c * SSM_T:(c + 1) * SSM_T]
        if j < nt - 1:
            b_q[c, j] = tuple(_dot(xb, bcat[o + j * LANES:o + (j + 1) * LANES, :], 0, 1) for o in (0, PM))
        else:
            bt = _dot(xb, bcat[2 * PM:, :], 0, 1)
            b_q[c, j] = (bt, pltpu.roll(bt, PR, 1))

    def ssm_window(c, j):
        br, bi = b_q.pop((c, j))
        ur, ui = tile(cr, j) * br - tile(ci, j) * bi, -(tile(cr, j) * bi + tile(ci, j) * br)
        yr = jnp.concatenate([tail[j][0], ur], axis=0)
        yi = jnp.concatenate([tail[j][1], ui], axis=0)
        tail[j] = (ur[SSM_T - 8:], ui[SSM_T - 8:])
        for sh, a in ((1, a1), (2, a2), (4, a4)):
            dr, di = _cmul(pltpu.roll(yr, sh, 0), pltpu.roll(yi, sh, 0), tile(a[0], j), tile(a[1], j))
            yr, yi = yr + dr, yi + di
        y_q[c, j] = (yr, yi)

    def ssm_scan(c, j):
        yr, yi = y_q.pop((c, j))
        hr, hi = state[j]
        hs = []
        for i in range(8, SSM_T + 8, 8):
            pr, pi = _cmul(hr, hi, tile(a8[0], j), tile(a8[1], j))
            hr, hi = pr + yr[i:i + 8], pi + yi[i:i + 8]
            hs.append((hr, hi))
        state[j] = (hr, hi)
        hr, hi = (jnp.concatenate(z, axis=0) for z in zip(*hs))
        if j < nt - 1:
            h_q[c, j] = (hr.astype(BF16), hi.astype(BF16))
        else:
            h_q[c, j] = jnp.where(low_half, hr, pltpu.roll(hi, PR, 1)).astype(BF16)

    def ssm_out(c):
        cols = slice(c * SSM_T, (c + 1) * SSM_T)
        hs = [h_q.pop((c, j)) for j in range(nt)]
        hcat = jnp.concatenate([z[0] for z in hs[:-1]] + [z[1] for z in hs[:-1]] + hs[-1:], axis=1)
        xf = xt[:, cols].astype(F32)
        y = _dot(ccat[...], hcat, 1, 1) + xf * dsk
        g = jax.nn.sigmoid(jnp.sum(xf * gw, axis=0, keepdims=True))
        g_s[:, cols] = g
        acc[:, cols] = (1.0 - g) * y

    for c in range(nc + 2):
        if c == 1:
            x_rest.wait()
        lanes = []
        if c < nc:
            lanes.append([functools.partial(ssm_in, c, j) for j in range(nt)])
        if 2 <= c:
            lanes.append([functools.partial(ssm_out, c - 2)])
        if 1 <= c <= nc:
            lanes.append([functools.partial(f, c - 1, j) for j in range(nt) for f in (ssm_window, ssm_scan)])
        interleave(lanes)

    def out_copy(i):
        cols = pl.ds(i * BQ, BQ)
        return pltpu.make_async_copy(acc.at[:, cols], out_hbm.at[:, cols], osems.at[i])

    def attend(h):
        slot = 0
        kj = jax.lax.broadcasted_iota(jnp.int32, (QT, QT), 0)
        qi = jax.lax.broadcasted_iota(jnp.int32, (QT, QT), 1)
        causal = kj <= qi

        def chunks(t):
            hi = (t + 1) * QT
            return [(lo, min(lo + CK, hi)) for lo in range(0, hi, CK)]

        fold = lambda v, op: functools.reduce(op, [v[i:i + FR] for i in range(0, v.shape[0], FR)])
        s_q, m_q, p_q, l_q, c_q = {}, {}, {}, {}, {}

        def scores(t, lo, hi):
            s = _dot(k_s[slot, lo:hi, :], qt_s[slot, :, t * QT:(t + 1) * QT])
            if hi == (t + 1) * QT:
                d = hi - lo - QT
                sd = jnp.where(causal, s[d:], -1e9)
                s = jnp.concatenate([s[:d], sd], axis=0) if d else sd
            s_q[t, lo] = s
            m = fold(s, jnp.maximum)
            m_q[t] = jnp.maximum(m_q[t], m) if lo else m

        def weights(t, lo, hi):
            if lo == 0:
                m_q[t] = jnp.max(m_q[t], axis=0, keepdims=True)
            p = jnp.exp2(s_q.pop((t, lo)) - m_q[t])
            p_q[t, lo] = p.astype(BF16)
            l = fold(p, jnp.add)
            l_q[t] = l_q[t] + l if lo else l

        def context(t, lo, hi):
            c = _dot(vt_s[slot, :, lo:hi], p_q.pop((t, lo)))
            c_q[t] = c_q[t] + c if lo else c
            if hi == (t + 1) * QT:
                l = jnp.sum(l_q[t], axis=0, keepdims=True)
                c_q[t] = (c_q[t] * (g_s[:, t * QT:(t + 1) * QT] / l)).astype(BF16)

        def output(i):
            c = jnp.concatenate([c_q.pop(t) for t in range(i * per, (i + 1) * per)], axis=1)
            acc[:, i * BQ:(i + 1) * BQ] += _dot(wot[h % 2], c)
            if OM:
                out_copy(i).start(priority=1)

        n = S // QT
        per = BQ // QT
        order = ORDER
        finished = set()
        for step in range(n + SK3):
            lanes = []
            for skew, f in ((0, scores), (SK1, weights), (SK2, context)):
                if 0 <= step - skew < n:
                    t = order[step - skew]
                    lanes.append([functools.partial(f, t, *c) for c in chunks(t)])
            if 0 <= step - SK3 < n:
                t = order[step - SK3]
                finished.add(t)
                if all(u in finished for u in range(t // per * per, (t // per + 1) * per)):
                    lanes.append([functools.partial(output, t // per)])
            interleave(lanes)

    def head(h, _):
        @pl.when(h % 2 == 0)
        def _():
            hp = h // 2
            for cp in pair_copies(hp, hp % 2):
                cp.wait()

            @pl.when(hp + 1 < H // 2)
            def _():
                for cp in pair_copies(hp + 1, 1 - hp % 2):
                    cp.start()

        wo_copy(h).wait()

        @pl.when(h + 1 < H)
        def _():
            wo_copy(h + 1).start()

        @pl.when(h > (0 if OM else H))
        def _():
            for i in range(S // BQ):
                out_copy(i).wait()

        for f in project(h):
            f()
        attend(h)
        return 0

    ckv_copy.wait()
    jax.lax.fori_loop(0, H, head, 0)
    for i in range(0 if OM else S // BQ):
        out_copy(i).start()
    for i in range(S // BQ):
        out_copy(i).wait()


@jax.jit
def pallas_gated_mix__compressed_kv_cla__ssm_conv_s5__prompt_kernel(
    A_x: jax.Array,
    A_c_kv: jax.Array,
    A_w_q: jax.Array,
    A_w_uk: jax.Array,
    A_w_uv: jax.Array,
    A_w_o: jax.Array,
    B_x: jax.Array,
    B_Lambda_re: jax.Array,
    B_Lambda_im: jax.Array,
    B_B_re: jax.Array,
    B_B_im: jax.Array,
    B_C_re: jax.Array,
    B_C_im: jax.Array,
    B_log_dt: jax.Array,
    B_Dskip: jax.Array,
    gate_w: jax.Array,
):
    del B_x
    B, S, M = A_x.shape
    Dc, H, D = A_w_uk.shape
    assert B == 1 and A_c_kv.shape[1] == S
    vmem = pl.BlockSpec(memory_space=pltpu.VMEM)
    hbm = pl.BlockSpec(memory_space=pltpu.HBM)
    out_t = pl.pallas_call(
        _kernel,
        in_specs=[vmem] * 5 + [hbm] * 10,
        out_specs=hbm,
        out_shape=pltpu.HBM((M, S), F32),
        scratch_shapes=[
            pltpu.VMEM((M, S), BF16),
            pltpu.VMEM((2 * M, M), BF16),
            pltpu.VMEM((M, M), BF16),
            pltpu.VMEM((M, M), BF16),
            pltpu.VMEM((M, 2 * M), BF16),
            pltpu.VMEM((S, Dc), BF16),
            pltpu.VMEM((2, M, D), jnp.uint32),
            pltpu.VMEM((2, Dc, D), jnp.uint32),
            pltpu.VMEM((2, Dc, D), jnp.uint32),
            pltpu.VMEM((2, M, D), BF16),
            pltpu.VMEM((M, S), F32),
            pltpu.VMEM((1, S), F32),
            pltpu.VMEM((2, D, S), BF16),
            pltpu.VMEM((2, S, D), BF16),
            pltpu.VMEM((2, D, S), BF16),
            pltpu.VMEM((Dc, D), BF16),
            pltpu.VMEM((M, D), BF16),
            pltpu.VMEM((D, Dc), BF16),
            pltpu.SemaphoreType.DMA((9,)),
            pltpu.SemaphoreType.DMA((4, 2)),
            pltpu.SemaphoreType.DMA((S // BQ,)),
        ],
        compiler_params=pltpu.CompilerParams(vmem_limit_bytes=64 * 2**20),
    )(B_Lambda_re, B_Lambda_im, B_log_dt, B_Dskip, gate_w,
      A_x.reshape(S, M).T, B_B_re, B_B_im, B_C_re, B_C_im,
      A_c_kv.reshape(S, Dc), A_w_q, A_w_uk, A_w_uv, A_w_o.transpose(0, 2, 1))
    return out_t.T.reshape(B, S, M)
```
